```python
import os as _os
_os.environ.setdefault("JAX_PLATFORMS", "cpu")
import jax
import jax.numpy as jnp

def _softmax(x, axis=-1):
    return jax.nn.softmax(x, axis=axis)
def _gelu(x):
    return jax.nn.gelu(x, approximate=True)
def _silu(x):
    return jax.nn.silu(x)
def _sigmoid(x):
    return jax.nn.sigmoid(x)
def _layernorm(x, axis=-1, eps=1e-5):
    m = jnp.mean(x, axis=axis, keepdims=True)
    v = jnp.var(x, axis=axis, keepdims=True)
    return (x - m) / jnp.sqrt(v + eps)
def _scatter_add(tgt, idx, src, axis=0):
    return tgt.at[idx].add(src)
def _segment_sum(src, seg, n):
    return jax.ops.segment_sum(src, seg, n)
class _Rng:
    def __init__(self, key):
        self._k = key
    def _next(self):
        self._k, sub = jax.random.split(self._k)
        return sub
    def normal(self, shape):
        return jax.random.normal(self._next(), shape, dtype=jnp.bfloat16)
    def randint(self, lo, hi, shape):
        return jax.random.randint(self._next(), shape, lo, hi, dtype=jnp.int32)
    def uniform(self, shape, lo=0.0, hi=1.0):
        return jax.random.uniform(self._next(), shape, jnp.bfloat16, lo, hi)
    def permutation(self, n):
        return jax.random.permutation(self._next(), n)


kernel_name = 'sequential_preLN__spectral_gfnet__glu_gated_bilinear__prompt'

def setup_inputs():
    _rng = _Rng(jax.random.key(int.from_bytes(__import__("os").urandom(4), "little")))
    _w = (lambda a: (lambda t: t.astype(jnp.bfloat16) if jnp.issubdtype(t.dtype, jnp.floating) else t)(jnp.asarray(a)))
    def _A_setup():
        B, S, D = 1, 2048, 448
        Df = D // 2 + 1
        return {
            "x": _w((lambda *s: _rng.normal(s) * 0.05)(B, S, D)),
            "w_r": _w((lambda *s: _rng.normal(s) * 0.2)(S, Df) * 0.02),
            "w_i": _w((lambda *s: _rng.normal(s) * 0.2)(S, Df) * 0.02),
        }
    _A_in = _A_setup()

    def _B_setup():
        B, S, D, F = 1, 2048, 448, 1792
        return {
            "x": _w((lambda *s: _rng.normal(s) * 0.05)(B, S, D)),
            "w_gate": _w((lambda *s: _rng.normal(s) * 0.05)(D, F) * (D ** -0.5)),
            "w_up": _w((lambda *s: _rng.normal(s) * 0.05)(D, F) * (D ** -0.5)),
            "w_down": _w((lambda *s: _rng.normal(s) * 0.05)(F, D) * (F ** -0.5)),
        }
    _B_in = _B_setup()

    return {
        "A_x": _A_in["x"],
        "A_w_r": _A_in["w_r"],
        "A_w_i": _A_in["w_i"],
        "B_x": _B_in["x"],
        "B_w_gate": _B_in["w_gate"],
        "B_w_up": _B_in["w_up"],
        "B_w_down": _B_in["w_down"],
    }

def reference(A_x, A_w_r, A_w_i, B_x, B_w_gate, B_w_up, B_w_down):
    def _A_ref(x, w_r, w_i):
        B, S, D = x.shape
        X = (lambda x, axes=(-2,-1): jnp.fft.rfft2(x.astype(jnp.float32), axes=axes))(x, axes=(-2, -1))
        W = w_r + 1j * w_i
        X = X * W
        y = (lambda x, s, axes=(-2,-1): jnp.fft.irfft2(x, s=s, axes=axes).astype(jnp.bfloat16))(X, (S, D), axes=(-2, -1))
        return y

    def _B_ref(x, w_gate, w_up, w_down):
        g = jnp.einsum("bsd,df->bsf", x, w_gate)
        u = jnp.einsum("bsd,df->bsf", x, w_up)
        h = g * u
        return jnp.einsum("bsf,fd->bsd", h, w_down)

    x = A_x
    h = x + _A_ref(_layernorm(x, axis=-1), A_w_r, A_w_i)
    h2 = h + _B_ref(_layernorm(h, axis=-1), B_w_gate, B_w_up, B_w_down)
    return h2
```

```python
import math
import numpy as np
import jax, jax.numpy as jnp
import jax.experimental.pallas as pl
import jax.experimental.pallas.tpu as pltpu

S, D, F = 2048, 448, 1792
DF = 225
DFP = 256
N1, N2 = 16, 128
TM1 = 256
TM3 = 256
EPS = 1e-5


def _fft16(xr, xi, sign):
    n = len(xr)
    if n == 1:
        return xr, xi
    er, ei = _fft16(xr[0::2], xi[0::2], sign)
    orr, oi = _fft16(xr[1::2], xi[1::2], sign)
    outr = [None] * n
    outi = [None] * n
    for k in range(n // 2):
        if k == 0:
            tr, ti = orr[k], oi[k]
        elif 4 * k == n:
            if sign < 0:
                tr, ti = oi[k], -orr[k]
            else:
                tr, ti = -oi[k], orr[k]
        else:
            c = math.cos(2 * math.pi * k / n)
            s = sign * math.sin(2 * math.pi * k / n)
            tr = orr[k] * c - oi[k] * s
            ti = orr[k] * s + oi[k] * c
        outr[k] = er[k] + tr
        outi[k] = ei[k] + ti
        outr[k + n // 2] = er[k] - tr
        outi[k + n // 2] = ei[k] - ti
    return outr, outi


def _ln(x):
    m = jnp.mean(x, axis=-1, keepdims=True)
    xc = x - m
    v = jnp.mean(xc * xc, axis=-1, keepdims=True)
    return xc * jax.lax.rsqrt(v + EPS)


def _cs(num, den):
    ang = num.astype(jnp.float32) * (2.0 * math.pi / den)
    return jnp.cos(ang), jnp.sin(ang)


def kernel(xt_hbm, wrt_hbm, wit_hbm, wg_hbm, wu_hbm, wdt_hbm, ot_hbm,
           X_scr, w_scr, fd_scr, id_scr, x_scr,
           xt_ref, wrt_ref, wit_ref, wg_ref, wu_ref, wdt_ref, ot_buf, sems, osems):
    cps = [pltpu.make_async_copy(src, dst, sems.at[i]) for i, (src, dst) in enumerate(
        [(xt_hbm, xt_ref), (wrt_hbm, wrt_ref), (wit_hbm, wit_ref), (wg_hbm, wg_ref), (wu_hbm, wu_ref), (wdt_hbm, wdt_ref)])]
    for cp in cps:
        cp.start()
    d_i = jax.lax.broadcasted_iota(jnp.int32, (D, DFP), 0)
    k_i = jax.lax.broadcasted_iota(jnp.int32, (D, DFP), 1)
    c, s = _cs((d_i * k_i) % D, D)
    valid = k_i < DF
    fd_scr[:, 0:DFP] = jnp.where(valid, c, 0.0).astype(jnp.bfloat16)
    fd_scr[:, DFP:2 * DFP] = jnp.where(valid, -s, 0.0).astype(jnp.bfloat16)
    k_i = jax.lax.broadcasted_iota(jnp.int32, (DFP, D), 0)
    d_i = jax.lax.broadcasted_iota(jnp.int32, (DFP, D), 1)
    c, s = _cs((d_i * k_i) % D, D)
    coef = jnp.where(k_i >= DF, 0.0, jnp.where((k_i == 0) | (k_i == DF - 1), 1.0, 2.0)) * (1.0 / (S * D))
    id_scr[0:DFP, :] = (c * coef).astype(jnp.bfloat16)
    id_scr[DFP:2 * DFP, :] = (-s * coef).astype(jnp.bfloat16)

    cps[1].wait()
    cps[2].wait()
    def wt(i, carry):
        r0 = pl.multiple_of(i * 256, 256)
        for j, ref in ((0, wrt_ref), (2, wit_ref)):
            a = ref[0:128, pl.ds(r0, 256)].astype(jnp.float32)
            w_scr[j, pl.ds(r0, 256), :] = a.T
            b = ref[128:DF, pl.ds(r0, 256)].astype(jnp.float32)
            b = jnp.concatenate([b, jnp.zeros((256 - DF, 256), jnp.float32)], axis=0)
            w_scr[j + 1, pl.ds(r0, 256), :] = b.T
        return carry
    jax.lax.fori_loop(0, S // 256, wt, 0)

    cps[0].wait()
    def p1(i, carry):
        r0 = pl.multiple_of(i * TM1, TM1)
        xb = xt_ref[:, pl.ds(r0, TM1)].astype(jnp.float32).T
        x_scr[pl.ds(r0, TM1), :] = xb.astype(jnp.bfloat16)
        xn = _ln(xb).astype(jnp.bfloat16)
        X_scr[pl.ds(r0, TM1), :] = jnp.dot(xn, fd_scr[...], preferred_element_type=jnp.float32)
        return carry
    jax.lax.fori_loop(0, S // TM1, p1, 0)

    def fft_pass(sign):
        def body(t, carry):
            r = pl.multiple_of((t // 2) * 8, 8)
            l = (t % 2) * 128
            l = pl.multiple_of(l, 128)
            xr = [X_scr[pl.ds(N2 * b + r, 8), pl.ds(l, 128)] for b in range(N1)]
            xi = [X_scr[pl.ds(N2 * b + r, 8), pl.ds(DFP + l, 128)] for b in range(N1)]
            yr, yi = _fft16(xr, xi, sign)
            for b in range(N1):
                X_scr[pl.ds(N2 * b + r, 8), pl.ds(l, 128)] = yr[b]
                X_scr[pl.ds(N2 * b + r, 8), pl.ds(DFP + l, 128)] = yi[b]
            return carry
        jax.lax.fori_loop(0, 2 * N2 // 8, body, 0)
    fft_pass(-1)

    a_i = jax.lax.broadcasted_iota(jnp.int32, (N2, N2), 0)
    b_i = jax.lax.broadcasted_iota(jnp.int32, (N2, N2), 1)
    fc, fs = _cs((a_i * b_i) % N2, N2)
    k16 = jax.lax.broadcasted_iota(jnp.int32, (N1, N2), 0)
    s16 = jax.lax.broadcasted_iota(jnp.int32, (N1, N2), 1)
    tc, ts = _cs(k16 * s16, S)
    s16 = jax.lax.broadcasted_iota(jnp.int32, (N2, N1), 0)
    k16 = jax.lax.broadcasted_iota(jnp.int32, (N2, N1), 1)
    tcT, tsT = _cs(k16 * s16, S)

    for k1 in range(N1):
        r0 = k1 * N2
        tr = tc[k1:k1 + 1, :]
        ti = ts[k1:k1 + 1, :]
        gr = (fc * tr - fs * ti).astype(jnp.bfloat16)
        gn = (fc * ti + fs * tr).astype(jnp.bfloat16)
        G = jnp.concatenate([jnp.concatenate([gr, gn], axis=1),
                             jnp.concatenate([-gn, gr], axis=1)], axis=0)
        A = X_scr[r0:r0 + N2, :]
        A2 = jnp.concatenate([A[:, :DFP], A[:, DFP:]], axis=0).astype(jnp.bfloat16)
        Y = jnp.dot(G, A2, preferred_element_type=jnp.float32)
        yr, yi = Y[:N2], Y[N2:]
        wv = [w_scr[j, pl.ds(k1, N2, stride=N1), :] for j in range(4)]
        wr = jnp.concatenate(wv[:2], axis=1)
        wi = jnp.concatenate(wv[2:], axis=1)
        zr = yr * wr - yi * wi
        zi = yr * wi + yi * wr
        Z2 = jnp.concatenate([zr, zi], axis=0).astype(jnp.bfloat16)
        trc = tcT[:, k1:k1 + 1]
        tic = tsT[:, k1:k1 + 1]
        hr = (fc * trc - fs * tic).astype(jnp.bfloat16)
        hi = (fc * tic + fs * trc).astype(jnp.bfloat16)
        H = jnp.concatenate([jnp.concatenate([hr, -hi], axis=1),
                             jnp.concatenate([hi, hr], axis=1)], axis=0)
        Bv = jnp.dot(H, Z2, preferred_element_type=jnp.float32)
        X_scr[r0:r0 + N2, 0:DFP] = Bv[:N2]
        X_scr[r0:r0 + N2, DFP:2 * DFP] = Bv[N2:]

    fft_pass(+1)

    for cp in cps[3:]:
        cp.wait()
    def ocp(i, slot):
        r0 = pl.multiple_of(i * TM3, TM3)
        return pltpu.make_async_copy(ot_buf.at[slot], ot_hbm.at[:, pl.ds(r0, TM3)], osems.at[slot])
    def p3(i, carry):
        r0 = pl.multiple_of(i * TM3, TM3)
        Yb = X_scr[pl.ds(r0, TM3), :].astype(jnp.bfloat16)
        y = jnp.dot(Yb, id_scr[...], preferred_element_type=jnp.float32)
        xb = x_scr[pl.ds(r0, TM3), :].astype(jnp.float32)
        h = (xb + y.astype(jnp.bfloat16).astype(jnp.float32)).astype(jnp.bfloat16).astype(jnp.float32)
        hn = _ln(h).astype(jnp.bfloat16)
        g = jnp.dot(hn, wg_ref[...], preferred_element_type=jnp.float32)
        u = jnp.dot(hn, wu_ref[...], preferred_element_type=jnp.float32)
        hh = (g * u).astype(jnp.bfloat16)
        o = jax.lax.dot_general(hh, wdt_ref[...], (((1,), (1,)), ((), ())), preferred_element_type=jnp.float32)
        slot = i % 2
        @pl.when(i >= 2)
        def _():
            ocp(i - 2, slot).wait()
        ot_buf[slot] = (h + o).T.astype(jnp.bfloat16)
        ocp(i, slot).start()
        return carry
    n3 = S // TM3
    jax.lax.fori_loop(0, n3, p3, 0)
    ocp(n3 - 2, (n3 - 2) % 2).wait()
    ocp(n3 - 1, (n3 - 1) % 2).wait()


@jax.jit
def pallas_sequential_preLN__spectral_gfnet__glu_gated_bilinear__prompt_kernel(A_x, A_w_r, A_w_i, B_x, B_w_gate, B_w_up, B_w_down):
    xt = A_x.reshape(S, D).T
    out = pl.pallas_call(
        kernel,
        out_shape=jax.ShapeDtypeStruct((D, S), jnp.bfloat16),
        scratch_shapes=[
            pltpu.VMEM((S, 2 * DFP), jnp.float32),
            pltpu.VMEM((4, S, 128), jnp.float32),
            pltpu.VMEM((D, 2 * DFP), jnp.bfloat16),
            pltpu.VMEM((2 * DFP, D), jnp.bfloat16),
            pltpu.VMEM((S, D), jnp.bfloat16),
            pltpu.VMEM((D, S), jnp.bfloat16),
            pltpu.VMEM((DF, S), jnp.bfloat16),
            pltpu.VMEM((DF, S), jnp.bfloat16),
            pltpu.VMEM((D, F), jnp.bfloat16),
            pltpu.VMEM((D, F), jnp.bfloat16),
            pltpu.VMEM((D, F), jnp.bfloat16),
            pltpu.VMEM((2, D, TM3), jnp.bfloat16),
            pltpu.SemaphoreType.DMA((6,)),
            pltpu.SemaphoreType.DMA((2,)),
        ],
        in_specs=[pl.BlockSpec(memory_space=pl.ANY)] * 6,
        out_specs=pl.BlockSpec(memory_space=pl.ANY),
        compiler_params=pltpu.CompilerParams(vmem_limit_bytes=100 * 1024 * 1024),
    )(xt, A_w_r.T, A_w_i.T, B_w_gate, B_w_up, B_w_down.T)
    return out.T.reshape(1, S, D)
```

```python
import math
import numpy as np
import jax, jax.numpy as jnp
import jax.experimental.pallas as pl
import jax.experimental.pallas.tpu as pltpu

S, D, F = 2048, 448, 1792
DF = 225
DFP = 256
N1, N2 = 16, 128
TM1 = 512
TM3 = 1024
EPS = 1e-5


def _fft16(xr, xi, sign):
    n = len(xr)
    if n == 1:
        return xr, xi
    er, ei = _fft16(xr[0::2], xi[0::2], sign)
    orr, oi = _fft16(xr[1::2], xi[1::2], sign)
    outr = [None] * n
    outi = [None] * n
    for k in range(n // 2):
        if k == 0:
            tr, ti = orr[k], oi[k]
        elif 4 * k == n:
            if sign < 0:
                tr, ti = oi[k], -orr[k]
            else:
                tr, ti = -oi[k], orr[k]
        else:
            c = math.cos(2 * math.pi * k / n)
            s = sign * math.sin(2 * math.pi * k / n)
            tr = orr[k] * c - oi[k] * s
            ti = orr[k] * s + oi[k] * c
        outr[k] = er[k] + tr
        outi[k] = ei[k] + ti
        outr[k + n // 2] = er[k] - tr
        outi[k + n // 2] = ei[k] - ti
    return outr, outi


def _ln(x):
    m = jnp.mean(x, axis=-1, keepdims=True)
    xc = x - m
    v = jnp.mean(xc * xc, axis=-1, keepdims=True)
    return xc * jax.lax.rsqrt(v + EPS)


def _cs(num, den):
    ang = num.astype(jnp.float32) * (2.0 * math.pi / den)
    return jnp.cos(ang), jnp.sin(ang)


def kernel(xt_hbm, wrt_hbm, wit_hbm, wg_hbm, wu_hbm, wdt_hbm, ot_hbm,
           X_scr, w_scr, fd_scr, id_scr, x_scr,
           xt_ref, wrt_ref, wit_ref, wg_ref, wu_ref, wdt_ref, ot_buf, sems, osems):
    cps = [pltpu.make_async_copy(src, dst, sems.at[i]) for i, (src, dst) in enumerate(
        [(xt_hbm, xt_ref), (wrt_hbm, wrt_ref), (wit_hbm, wit_ref), (wg_hbm, wg_ref), (wu_hbm, wu_ref), (wdt_hbm, wdt_ref)])]
    for cp in cps:
        cp.start()
    d_i = jax.lax.broadcasted_iota(jnp.int32, (D, DFP), 0)
    k_i = jax.lax.broadcasted_iota(jnp.int32, (D, DFP), 1)
    c, s = _cs((d_i * k_i) % D, D)
    valid = k_i < DF
    fd_scr[:, 0:DFP] = jnp.where(valid, c, 0.0).astype(jnp.bfloat16)
    fd_scr[:, DFP:2 * DFP] = jnp.where(valid, -s, 0.0).astype(jnp.bfloat16)
    k_i = jax.lax.broadcasted_iota(jnp.int32, (DFP, D), 0)
    d_i = jax.lax.broadcasted_iota(jnp.int32, (DFP, D), 1)
    c, s = _cs((d_i * k_i) % D, D)
    coef = jnp.where(k_i >= DF, 0.0, jnp.where((k_i == 0) | (k_i == DF - 1), 1.0, 2.0)) * (1.0 / (S * D))
    id_scr[0:DFP, :] = (c * coef).astype(jnp.bfloat16)
    id_scr[DFP:2 * DFP, :] = (-s * coef).astype(jnp.bfloat16)

    cps[1].wait()
    cps[2].wait()
    def wt(i, carry):
        r0 = pl.multiple_of(i * 256, 256)
        for j, ref in ((0, wrt_ref), (2, wit_ref)):
            a = ref[0:128, pl.ds(r0, 256)].astype(jnp.float32)
            w_scr[j, pl.ds(r0, 256), :] = a.T
            b = ref[128:DF, pl.ds(r0, 256)].astype(jnp.float32)
            b = jnp.concatenate([b, jnp.zeros((256 - DF, 256), jnp.float32)], axis=0)
            w_scr[j + 1, pl.ds(r0, 256), :] = b.T
        return carry
    jax.lax.fori_loop(0, S // 256, wt, 0)

    cps[0].wait()
    def p1(i, carry):
        r0 = pl.multiple_of(i * TM1, TM1)
        V = 'c'
        if V == 'a':
            xb = xt_ref[:, pl.ds(r0, TM1)].astype(jnp.float32).T
            x_scr[pl.ds(r0, TM1), :] = xb.astype(jnp.bfloat16)
            xn = _ln(xb).astype(jnp.bfloat16)
        elif V == 'b':
            xb16 = xt_ref[:, pl.ds(r0, TM1)].T
            x_scr[pl.ds(r0, TM1), :] = xb16
            xn = _ln(xb16.astype(jnp.float32)).astype(jnp.bfloat16)
        elif V == 'c':
            xt16 = xt_ref[:, pl.ds(r0, TM1)]
            xt = xt16.astype(jnp.float32)
            m = jnp.mean(xt, axis=0, keepdims=True)
            xc = xt - m
            v = jnp.mean(xc * xc, axis=0, keepdims=True)
            xn = (xc * jax.lax.rsqrt(v + 1e-5)).astype(jnp.bfloat16).T
            x_scr[pl.ds(r0, TM1), :] = xt16.T
        X_scr[pl.ds(r0, TM1), :] = jnp.dot(xn, fd_scr[...], preferred_element_type=jnp.float32)
        return carry
    jax.lax.fori_loop(0, S // TM1, p1, 0)

    def fft_pass(sign):
        def body(t, carry):
            FR = 8; FL = 256
            nl = DFP // FL
            r = pl.multiple_of((t // nl) * FR, FR)
            l = (t % nl) * FL
            l = pl.multiple_of(l, FL)
            xr = [X_scr[pl.ds(N2 * b + r, FR), pl.ds(l, FL)] for b in range(N1)]
            xi = [X_scr[pl.ds(N2 * b + r, FR), pl.ds(DFP + l, FL)] for b in range(N1)]
            yr, yi = _fft16(xr, xi, sign)
            for b in range(N1):
                X_scr[pl.ds(N2 * b + r, FR), pl.ds(l, FL)] = yr[b]
                X_scr[pl.ds(N2 * b + r, FR), pl.ds(DFP + l, FL)] = yi[b]
            return carry
        FR = 8; FL = 256
        jax.lax.fori_loop(0, (DFP // FL) * N2 // FR, body, 0)
    fft_pass(-1)

    a_i = jax.lax.broadcasted_iota(jnp.int32, (N2, N2), 0)
    b_i = jax.lax.broadcasted_iota(jnp.int32, (N2, N2), 1)
    fc, fs = _cs((a_i * b_i) % N2, N2)
    k16 = jax.lax.broadcasted_iota(jnp.int32, (N1, N2), 0)
    s16 = jax.lax.broadcasted_iota(jnp.int32, (N1, N2), 1)
    tc, ts = _cs(k16 * s16, S)
    s16 = jax.lax.broadcasted_iota(jnp.int32, (N2, N1), 0)
    k16 = jax.lax.broadcasted_iota(jnp.int32, (N2, N1), 1)
    tcT, tsT = _cs(k16 * s16, S)

    for k1 in range(N1):
        r0 = k1 * N2
        tr = tc[k1:k1 + 1, :]
        ti = ts[k1:k1 + 1, :]
        gr = (fc * tr - fs * ti).astype(jnp.bfloat16)
        gn = (fc * ti + fs * tr).astype(jnp.bfloat16)
        G = jnp.concatenate([jnp.concatenate([gr, gn], axis=1),
                             jnp.concatenate([-gn, gr], axis=1)], axis=0)
        A = X_scr[r0:r0 + N2, :]
        A2 = jnp.concatenate([A[:, :DFP], A[:, DFP:]], axis=0).astype(jnp.bfloat16)
        Y = jnp.dot(G, A2, preferred_element_type=jnp.float32)
        yr, yi = Y[:N2], Y[N2:]
        wv = [w_scr[j, pl.ds(k1, N2, stride=N1), :] for j in range(4)]
        wr = jnp.concatenate(wv[:2], axis=1)
        wi = jnp.concatenate(wv[2:], axis=1)
        zr = yr * wr - yi * wi
        zi = yr * wi + yi * wr
        Z2 = jnp.concatenate([zr, zi], axis=0).astype(jnp.bfloat16)
        trc = tcT[:, k1:k1 + 1]
        tic = tsT[:, k1:k1 + 1]
        hr = (fc * trc - fs * tic).astype(jnp.bfloat16)
        hi = (fc * tic + fs * trc).astype(jnp.bfloat16)
        H = jnp.concatenate([jnp.concatenate([hr, -hi], axis=1),
                             jnp.concatenate([hi, hr], axis=1)], axis=0)
        Bv = jnp.dot(H, Z2, preferred_element_type=jnp.float32)
        X_scr[r0:r0 + N2, 0:DFP] = Bv[:N2]
        X_scr[r0:r0 + N2, DFP:2 * DFP] = Bv[N2:]

    fft_pass(+1)

    for cp in cps[3:]:
        cp.wait()
    def ocp(i, slot):
        r0 = pl.multiple_of(i * TM3, TM3)
        return pltpu.make_async_copy(ot_buf.at[slot], ot_hbm.at[:, pl.ds(r0, TM3)], osems.at[slot])
    def p3(i, carry):
        r0 = pl.multiple_of(i * TM3, TM3)
        Yb = X_scr[pl.ds(r0, TM3), :].astype(jnp.bfloat16)
        y = jnp.dot(Yb, id_scr[...], preferred_element_type=jnp.float32)
        xb = x_scr[pl.ds(r0, TM3), :].astype(jnp.float32)
        h = (xb + y.astype(jnp.bfloat16).astype(jnp.float32)).astype(jnp.bfloat16).astype(jnp.float32)
        hn = _ln(h).astype(jnp.bfloat16)
        g = jnp.dot(hn, wg_ref[...], preferred_element_type=jnp.float32)
        u = jnp.dot(hn, wu_ref[...], preferred_element_type=jnp.float32)
        hh = (g * u).astype(jnp.bfloat16)
        o = jax.lax.dot_general(hh, wdt_ref[...], (((1,), (1,)), ((), ())), preferred_element_type=jnp.float32)
        slot = i % 2
        @pl.when(i >= 2)
        def _():
            ocp(i - 2, slot).wait()
        ot_buf[slot] = (h + o).T.astype(jnp.bfloat16)
        ocp(i, slot).start()
        return carry
    n3 = S // TM3
    jax.lax.fori_loop(0, n3, p3, 0)
    ocp(n3 - 2, (n3 - 2) % 2).wait()
    ocp(n3 - 1, (n3 - 1) % 2).wait()


@jax.jit
def pallas_sequential_preLN__spectral_gfnet__glu_gated_bilinear__prompt_kernel(A_x, A_w_r, A_w_i, B_x, B_w_gate, B_w_up, B_w_down):
    xt = A_x.reshape(S, D).T
    out = pl.pallas_call(
        kernel,
        out_shape=jax.ShapeDtypeStruct((D, S), jnp.bfloat16),
        scratch_shapes=[
            pltpu.VMEM((S, 2 * DFP), jnp.float32),
            pltpu.VMEM((4, S, 128), jnp.float32),
            pltpu.VMEM((D, 2 * DFP), jnp.bfloat16),
            pltpu.VMEM((2 * DFP, D), jnp.bfloat16),
            pltpu.VMEM((S, D), jnp.bfloat16),
            pltpu.VMEM((D, S), jnp.bfloat16),
            pltpu.VMEM((DF, S), jnp.bfloat16),
            pltpu.VMEM((DF, S), jnp.bfloat16),
            pltpu.VMEM((D, F), jnp.bfloat16),
            pltpu.VMEM((D, F), jnp.bfloat16),
            pltpu.VMEM((D, F), jnp.bfloat16),
            pltpu.VMEM((2, D, TM3), jnp.bfloat16),
            pltpu.SemaphoreType.DMA((6,)),
            pltpu.SemaphoreType.DMA((2,)),
        ],
        in_specs=[pl.BlockSpec(memory_space=pl.ANY)] * 6,
        out_specs=pl.BlockSpec(memory_space=pl.ANY),
        compiler_params=pltpu.CompilerParams(vmem_limit_bytes=100 * 1024 * 1024),
    )(xt, A_w_r.T, A_w_i.T, B_w_gate, B_w_up, B_w_down.T)
    return out.T.reshape(1, S, D)
```
